```python
import os as _os
_os.environ.setdefault("JAX_PLATFORMS", "cpu")
import jax
import jax.numpy as jnp

def _softmax(x, axis=-1):
    return jax.nn.softmax(x, axis=axis)
def _gelu(x):
    return jax.nn.gelu(x, approximate=True)
def _silu(x):
    return jax.nn.silu(x)
def _sigmoid(x):
    return jax.nn.sigmoid(x)
def _layernorm(x, axis=-1, eps=1e-5):
    m = jnp.mean(x, axis=axis, keepdims=True)
    v = jnp.var(x, axis=axis, keepdims=True)
    return (x - m) / jnp.sqrt(v + eps)
def _scatter_add(tgt, idx, src, axis=0):
    return tgt.at[idx].add(src)
def _segment_sum(src, seg, n):
    return jax.ops.segment_sum(src, seg, n)
class _Rng:
    def __init__(self, key):
        self._k = key
    def _next(self):
        self._k, sub = jax.random.split(self._k)
        return sub
    def normal(self, shape):
        return jax.random.normal(self._next(), shape, dtype=jnp.bfloat16)
    def randint(self, lo, hi, shape):
        return jax.random.randint(self._next(), shape, lo, hi, dtype=jnp.int32)
    def uniform(self, shape, lo=0.0, hi=1.0):
        return jax.random.uniform(self._next(), shape, jnp.bfloat16, lo, hi)
    def permutation(self, n):
        return jax.random.permutation(self._next(), n)


kernel_name = 'concat_heads__sliding_local_dilated__sliding_block__prompt'

def setup_inputs():
    _rng = _Rng(jax.random.key(int.from_bytes(__import__("os").urandom(4), "little")))
    _w = (lambda a: (lambda t: t.astype(jnp.bfloat16) if jnp.issubdtype(t.dtype, jnp.floating) else t)(jnp.asarray(a)))
    def _A_setup():
        B, S, D = 1, 2048, 1024
        return {
            "x": _w((lambda *s: _rng.normal(s) * 0.2)(B, S, D)),
            "wqkv": _w((lambda *s: _rng.normal(s) * 0.2)(D, 3 * D)),
            "wo": _w((lambda *s: _rng.normal(s) * 0.05)(D, D)),
        }
    _A_in = _A_setup()

    def _B_setup():
        B, S, D = 1, 2048, 1024
        return {
            "x": _w((lambda *s: _rng.normal(s) * 0.2)(B, S, D)),
            "wqkv": _w((lambda *s: _rng.normal(s) * 0.2)(D, 3 * D)),
            "wo": _w((lambda *s: _rng.normal(s) * 0.05)(D, D)),
        }
    _B_in = _B_setup()

    return {
        "A_x": _A_in["x"],
        "A_wqkv": _A_in["wqkv"],
        "A_wo": _A_in["wo"],
        "B_x": _B_in["x"],
        "B_wqkv": _B_in["wqkv"],
        "B_wo": _B_in["wo"],
    }

def reference(A_x, A_wqkv, A_wo, B_x, B_wqkv, B_wo):
    def _A_ref(x, wqkv, wo):
        B, S, D = x.shape
        H = 32; Dh = D // H
        W, dil = 8, 2
        qkv = (lambda x, *d: x.transpose(*d))((x @ wqkv).reshape(B, S, 3, H, Dh), 2, 0, 3, 1, 4)
        q, k, v = qkv[0], qkv[1], qkv[2]
        scale = Dh ** -0.5
        pos = jnp.arange(S)
        off = jnp.arange(W) * dil
        idx = pos[:, None] - off[None, :]
        mask = idx >= 0
        idx_c = jnp.where(mask, idx, 0).reshape(-1)
        kg = k[:, :, idx_c, :].reshape(B, H, S, W, Dh)
        vg = v[:, :, idx_c, :].reshape(B, H, S, W, Dh)
        logits = jnp.einsum("bhsd,bhswd->bhsw", q, kg) * scale
        logits = jnp.where(mask[None, None, :, :], logits, -1e9)
        attn = _softmax(logits, axis=-1)
        o = jnp.einsum("bhsw,bhswd->bhsd", attn, vg)
        return (lambda x, *d: x.transpose(*d))(o, 0, 2, 1, 3).reshape(B, S, D) @ wo

    def _B_ref(x, wqkv, wo):
        B, S, D = x.shape
        H = 32; Dh = D // H; W = 256
        qkv = (lambda x, *d: x.transpose(*d))((x @ wqkv).reshape(B, S, 3, H, Dh), 2, 0, 3, 1, 4)
        q, k, v = qkv[0], qkv[1], qkv[2]
        scores = jnp.einsum("bhqd,bhkd->bhqk", q, k) * (Dh ** -0.5)
        idx = jnp.arange(S)
        mask = (idx[:, None] - idx[None, :] >= 0) & (idx[:, None] - idx[None, :] < W)
        scores = jnp.where(mask[None, None], scores, -1e9)
        p = _softmax(scores, axis=-1)
        o = jnp.einsum("bhqk,bhkd->bhqd", p, v)
        return (lambda x, *d: x.transpose(*d))(o, 0, 2, 1, 3).reshape(B, S, D) @ wo

    a = _A_ref(A_x, A_wqkv, A_wo)
    b = _B_ref(B_x, B_wqkv, B_wo)
    return jnp.concatenate([a, b], axis=-1)
```

```python
import functools

import jax
import jax.numpy as jnp
from jax import lax
import jax.experimental.pallas as pl
import jax.experimental.pallas.tpu as pltpu

S = 2048
D = 1024
H = 32
DH = 32
BQ = 256
NG = D // 128
A_SUB = 64
A_PAD = 64
B_SUB = 128
B_PAD = 256
SCALE = DH ** -0.5
NEG = -1e9

_NT = (((1,), (1,)), ((), ()))
_NN = (((1,), (0,)), ((), ()))


def _lane_head_masks(rows):
    lane = lax.broadcasted_iota(jnp.int32, (rows, 128), 1)
    return [(lane // DH) == j for j in range(4)]


def _attend(q_g, k_g, v_g, valid, hmasks):
    R = q_g.shape[0]
    zero = jnp.zeros_like(q_g)
    q_stack = jnp.concatenate([jnp.where(hmasks[j], q_g, zero) for j in range(4)], axis=0)
    s = lax.dot_general(q_stack, k_g, _NT, preferred_element_type=jnp.float32)
    s = jnp.where(valid, s * SCALE, NEG)
    m = jnp.max(s, axis=-1, keepdims=True)
    p = jnp.exp(s - m)
    l = jnp.sum(p, axis=-1, keepdims=True)
    o = lax.dot_general(p.astype(jnp.bfloat16), v_g, _NN, preferred_element_type=jnp.float32)
    o = o * (1.0 / l)
    out = jnp.where(hmasks[0], o[0:R], 0.0)
    for j in range(1, 4):
        out = jnp.where(hmasks[j], o[j * R:(j + 1) * R], out)
    return out


def _kernel(xa_ref, xb_ref, wqa_ref, woa_ref, wqb_ref, wob_ref, out_ref,
            kva_scr, kvb_scr, oa_scr, ob_scr):
    i = pl.program_id(0)

    @pl.when(i == 0)
    def _():
        kva_scr[0:A_PAD, :] = jnp.zeros((A_PAD, 2 * D), jnp.bfloat16)
        kvb_scr[0:B_PAD, :] = jnp.zeros((B_PAD, 2 * D), jnp.bfloat16)

    row0 = pl.multiple_of(i * BQ, BQ)

    qkva = jnp.dot(xa_ref[...], wqa_ref[...], preferred_element_type=jnp.float32)
    qa = qkva[:, :D].astype(jnp.bfloat16)
    kva_scr[pl.ds(A_PAD + row0, BQ), :] = qkva[:, D:].astype(jnp.bfloat16)

    qkvb = jnp.dot(xb_ref[...], wqb_ref[...], preferred_element_type=jnp.float32)
    qb = qkvb[:, :D].astype(jnp.bfloat16)
    kvb_scr[pl.ds(B_PAD + row0, BQ), :] = qkvb[:, D:].astype(jnp.bfloat16)

    hm_a = _lane_head_masks(A_SUB)
    r = lax.broadcasted_iota(jnp.int32, (4 * A_SUB, 2 * A_SUB), 0) % A_SUB
    c = lax.broadcasted_iota(jnp.int32, (4 * A_SUB, 2 * A_SUB), 1)
    delta = r + A_SUB - c
    band_a = (delta >= 0) & (delta <= 14) & ((delta & 1) == 0)
    for sb in range(BQ // A_SUB):
        base = row0 + sb * A_SUB
        if sb == 0:
            valid = band_a & ((c + base - A_PAD) >= 0)
        else:
            valid = band_a
        for g in range(NG):
            q_g = qa[sb * A_SUB:(sb + 1) * A_SUB, g * 128:(g + 1) * 128]
            k_g = kva_scr[pl.ds(base, 2 * A_SUB), g * 128:(g + 1) * 128]
            v_g = kva_scr[pl.ds(base, 2 * A_SUB), D + g * 128:D + (g + 1) * 128]
            o = _attend(q_g, k_g, v_g, valid, hm_a)
            oa_scr[sb * A_SUB:(sb + 1) * A_SUB, g * 128:(g + 1) * 128] = o.astype(jnp.bfloat16)

    hm_b = _lane_head_masks(B_SUB)
    NK = 3 * B_SUB
    r = lax.broadcasted_iota(jnp.int32, (4 * B_SUB, NK), 0) % B_SUB
    c = lax.broadcasted_iota(jnp.int32, (4 * B_SUB, NK), 1)
    delta = r + 2 * B_SUB - c
    band_b = (delta >= 0) & (delta < 256)
    for sb in range(BQ // B_SUB):
        base = row0 + sb * B_SUB
        valid = band_b & ((c + base - B_PAD) >= 0)
        for g in range(NG):
            q_g = qb[sb * B_SUB:(sb + 1) * B_SUB, g * 128:(g + 1) * 128]
            k_g = kvb_scr[pl.ds(base, NK), g * 128:(g + 1) * 128]
            v_g = kvb_scr[pl.ds(base, NK), D + g * 128:D + (g + 1) * 128]
            o = _attend(q_g, k_g, v_g, valid, hm_b)
            ob_scr[sb * B_SUB:(sb + 1) * B_SUB, g * 128:(g + 1) * 128] = o.astype(jnp.bfloat16)

    out_ref[:, 0:D] = jnp.dot(oa_scr[...], woa_ref[...],
                              preferred_element_type=jnp.float32).astype(out_ref.dtype)
    out_ref[:, D:2 * D] = jnp.dot(ob_scr[...], wob_ref[...],
                                  preferred_element_type=jnp.float32).astype(out_ref.dtype)


@jax.jit
def pallas_concat_heads__sliding_local_dilated__sliding_block__prompt_kernel(
    A_x: jax.Array,
    A_wqkv: jax.Array,
    A_wo: jax.Array,
    B_x: jax.Array,
    B_wqkv: jax.Array,
    B_wo: jax.Array,
):
    xa = A_x.reshape(S, D)
    xb = B_x.reshape(S, D)

    def wspec(shape):
        return pl.BlockSpec(shape, lambda i: (0, 0), pipeline_mode=pl.Buffered(1))

    out = pl.pallas_call(
        _kernel,
        grid=(S // BQ,),
        in_specs=[
            pl.BlockSpec((BQ, D), lambda i: (i, 0)),
            pl.BlockSpec((BQ, D), lambda i: (i, 0)),
            wspec((D, 3 * D)),
            wspec((D, D)),
            wspec((D, 3 * D)),
            wspec((D, D)),
        ],
        out_specs=pl.BlockSpec((BQ, 2 * D), lambda i: (i, 0)),
        out_shape=jax.ShapeDtypeStruct((S, 2 * D), jnp.bfloat16),
        scratch_shapes=[
            pltpu.VMEM((A_PAD + S, 2 * D), jnp.bfloat16),
            pltpu.VMEM((B_PAD + S, 2 * D), jnp.bfloat16),
            pltpu.VMEM((BQ, D), jnp.bfloat16),
            pltpu.VMEM((BQ, D), jnp.bfloat16),
        ],
        compiler_params=pltpu.CompilerParams(
            dimension_semantics=("arbitrary",),
            vmem_limit_bytes=110 * 1024 * 1024,
        ),
    )(xa, xb, A_wqkv, A_wo, B_wqkv, B_wo)
    return out.reshape(1, S, 2 * D)
```

```python
import functools

import jax
import jax.numpy as jnp
from jax import lax
import jax.experimental.pallas as pl
import jax.experimental.pallas.tpu as pltpu

S = 2048
D = 1024
H = 32
DH = 32
BQ = 256
NG = D // 128
A_SUB = 64
A_PAD = 64
B_SUB = 128
B_PAD = 256
SCALE = DH ** -0.5
NEG = -1e9

_NT = (((1,), (1,)), ((), ()))
_NN = (((1,), (0,)), ((), ()))


def _lane_head_masks(rows):
    lane = lax.broadcasted_iota(jnp.int32, (rows, 128), 1)
    return [(lane // DH) == j for j in range(4)]


def _attend(q_g, k_g, v_g, valid, hmasks):
    R = q_g.shape[0]
    zero = jnp.zeros_like(q_g)
    q_stack = jnp.concatenate([jnp.where(hmasks[j], q_g, zero) for j in range(4)], axis=0)
    s = lax.dot_general(q_stack, k_g, _NT, preferred_element_type=jnp.float32)
    s = jnp.where(valid, s * SCALE, NEG)
    m = jnp.max(s, axis=-1, keepdims=True)
    p = jnp.exp(s - m)
    l = jnp.sum(p, axis=-1, keepdims=True)
    o = lax.dot_general(p.astype(jnp.bfloat16), v_g, _NN, preferred_element_type=jnp.float32)
    out = o[0:R]
    den = jnp.broadcast_to(l[0:R], (R, 128))
    for j in range(1, 4):
        out = jnp.where(hmasks[j], o[j * R:(j + 1) * R], out)
        den = jnp.where(hmasks[j], l[j * R:(j + 1) * R], den)
    inv = pl.reciprocal(den, approx=True)
    inv = inv * (2.0 - den * inv)
    return out * inv


def _attention(row0, out_ref, woa, wob, qkva, qkvb, oa_scr, ob_scr):
    hm_a = _lane_head_masks(A_SUB)
    r = lax.broadcasted_iota(jnp.int32, (4 * A_SUB, 2 * A_SUB), 0) % A_SUB
    c = lax.broadcasted_iota(jnp.int32, (4 * A_SUB, 2 * A_SUB), 1)
    delta = r + A_SUB - c
    band_a = (delta >= 0) & (delta <= 14) & ((delta & 1) == 0)
    for sb in range(BQ // A_SUB):
        base = row0 + sb * A_SUB
        if sb == 0:
            valid = band_a & ((c + base - A_PAD) >= 0)
        else:
            valid = band_a
        for g in range(NG):
            q_g = qkva[pl.ds(base + A_PAD, A_SUB), g * 128:(g + 1) * 128]
            k_g = qkva[pl.ds(base, 2 * A_SUB), D + g * 128:D + (g + 1) * 128]
            v_g = qkva[pl.ds(base, 2 * A_SUB), 2 * D + g * 128:2 * D + (g + 1) * 128]
            o = _attend(q_g, k_g, v_g, valid, hm_a)
            oa_scr[sb * A_SUB:(sb + 1) * A_SUB, g * 128:(g + 1) * 128] = o.astype(jnp.bfloat16)

    hm_b = _lane_head_masks(B_SUB)
    NK = 3 * B_SUB
    r = lax.broadcasted_iota(jnp.int32, (4 * B_SUB, NK), 0) % B_SUB
    c = lax.broadcasted_iota(jnp.int32, (4 * B_SUB, NK), 1)
    delta = r + 2 * B_SUB - c
    band_b = (delta >= 0) & (delta < 256)
    for sb in range(BQ // B_SUB):
        base = row0 + sb * B_SUB
        valid = band_b & ((c + base - B_PAD) >= 0)
        for g in range(NG):
            q_g = qkvb[pl.ds(base + B_PAD, B_SUB), g * 128:(g + 1) * 128]
            k_g = qkvb[pl.ds(base, NK), D + g * 128:D + (g + 1) * 128]
            v_g = qkvb[pl.ds(base, NK), 2 * D + g * 128:2 * D + (g + 1) * 128]
            o = _attend(q_g, k_g, v_g, valid, hm_b)
            ob_scr[sb * B_SUB:(sb + 1) * B_SUB, g * 128:(g + 1) * 128] = o.astype(jnp.bfloat16)

    out_ref[:, 0:D] = jnp.dot(oa_scr[...], woa[...],
                              preferred_element_type=jnp.float32).astype(out_ref.dtype)
    out_ref[:, D:2 * D] = jnp.dot(ob_scr[...], wob[...],
                                  preferred_element_type=jnp.float32).astype(out_ref.dtype)


def _kernel(xa_ref, xb_ref, wqa_hbm, woa_hbm, wqb_hbm, wob_hbm, out_ref,
            wqa, woa, wqb, wob, qkva, qkvb, oa_scr, ob_scr, sems):
    i = pl.program_id(0)
    row0 = pl.multiple_of(i * BQ, BQ)

    def wcopy(src, dst, n, t):
        cols = pl.ds(pl.multiple_of(t * D, D), D)
        return pltpu.make_async_copy(src.at[:, cols], dst.at[:, cols], sems.at[n + t])

    @pl.when(i == 0)
    def _():
        for t in range(3):
            wcopy(wqa_hbm, wqa, 0, t).start()
        for t in range(3):
            wcopy(wqb_hbm, wqb, 3, t).start()
        pltpu.make_async_copy(woa_hbm, woa, sems.at[6]).start()
        pltpu.make_async_copy(wob_hbm, wob, sems.at[7]).start()
        qkva[0:A_PAD, :] = jnp.zeros((A_PAD, 3 * D), jnp.bfloat16)
        qkvb[0:B_PAD, :] = jnp.zeros((B_PAD, 3 * D), jnp.bfloat16)

        def chunk_a(t, carry):
            wcopy(wqa_hbm, wqa, 0, t).wait()
            cols = pl.ds(pl.multiple_of(t * D, D), D)
            qkva[A_PAD:A_PAD + BQ, cols] = jnp.dot(
                xa_ref[...], wqa[:, cols], preferred_element_type=jnp.float32).astype(jnp.bfloat16)
            return carry

        lax.fori_loop(0, 3, chunk_a, 0)

        def chunk_b(t, carry):
            wcopy(wqb_hbm, wqb, 3, t).wait()
            cols = pl.ds(pl.multiple_of(t * D, D), D)
            qkvb[B_PAD:B_PAD + BQ, cols] = jnp.dot(
                xb_ref[...], wqb[:, cols], preferred_element_type=jnp.float32).astype(jnp.bfloat16)
            return carry

        lax.fori_loop(0, 3, chunk_b, 0)
        pltpu.make_async_copy(woa_hbm, woa, sems.at[6]).wait()
        pltpu.make_async_copy(wob_hbm, wob, sems.at[7]).wait()

    @pl.when(i > 0)
    def _():
        qkva[pl.ds(A_PAD + row0, BQ), :] = jnp.dot(
            xa_ref[...], wqa[...], preferred_element_type=jnp.float32).astype(jnp.bfloat16)
        qkvb[pl.ds(B_PAD + row0, BQ), :] = jnp.dot(
            xb_ref[...], wqb[...], preferred_element_type=jnp.float32).astype(jnp.bfloat16)

    _attention(row0, out_ref, woa, wob, qkva, qkvb, oa_scr, ob_scr)


@jax.jit
def pallas_concat_heads__sliding_local_dilated__sliding_block__prompt_kernel(
    A_x: jax.Array,
    A_wqkv: jax.Array,
    A_wo: jax.Array,
    B_x: jax.Array,
    B_wqkv: jax.Array,
    B_wo: jax.Array,
):
    xa = A_x.reshape(S, D)
    xb = B_x.reshape(S, D)

    out = pl.pallas_call(
        _kernel,
        grid=(S // BQ,),
        in_specs=[
            pl.BlockSpec((BQ, D), lambda i: (i, 0)),
            pl.BlockSpec((BQ, D), lambda i: (i, 0)),
            pl.BlockSpec(memory_space=pl.ANY),
            pl.BlockSpec(memory_space=pl.ANY),
            pl.BlockSpec(memory_space=pl.ANY),
            pl.BlockSpec(memory_space=pl.ANY),
        ],
        out_specs=pl.BlockSpec((BQ, 2 * D), lambda i: (i, 0)),
        out_shape=jax.ShapeDtypeStruct((S, 2 * D), jnp.bfloat16),
        scratch_shapes=[
            pltpu.VMEM((D, 3 * D), jnp.bfloat16),
            pltpu.VMEM((D, D), jnp.bfloat16),
            pltpu.VMEM((D, 3 * D), jnp.bfloat16),
            pltpu.VMEM((D, D), jnp.bfloat16),
            pltpu.VMEM((A_PAD + S, 3 * D), jnp.bfloat16),
            pltpu.VMEM((B_PAD + S, 3 * D), jnp.bfloat16),
            pltpu.VMEM((BQ, D), jnp.bfloat16),
            pltpu.VMEM((BQ, D), jnp.bfloat16),
            pltpu.SemaphoreType.DMA((8,)),
        ],
        compiler_params=pltpu.CompilerParams(
            dimension_semantics=("arbitrary",),
            vmem_limit_bytes=110 * 1024 * 1024,
        ),
    )(xa, xb, A_wqkv, A_wo, B_wqkv, B_wo)
    return out.reshape(1, S, 2 * D)
```
